```python
import jax
import jax.numpy as jnp

def _softmax(x, axis=-1):
    return jax.nn.softmax(x, axis=axis)

def _gelu(x):
    return jax.nn.gelu(x, approximate=True)

def _silu(x):
    return jax.nn.silu(x)

def _sigmoid(x):
    return jax.nn.sigmoid(x)

def _layernorm(x, axis=-1, eps=1e-05):
    m = jnp.mean(x, axis=axis, keepdims=True)
    v = jnp.var(x, axis=axis, keepdims=True)
    return (x - m) / jnp.sqrt(v + eps)

def _scatter_add(tgt, idx, src, axis=0):
    return tgt.at[idx].add(src)

def _segment_sum(src, seg, n):
    return jax.ops.segment_sum(src, seg, n)

class _Rng:

    def __init__(self, key):
        self._k = key

    def _next(self):
        self._k, sub = jax.random.split(self._k)
        return sub

    def normal(self, shape):
        return jax.random.normal(self._next(), shape, dtype=jnp.bfloat16)

    def randint(self, lo, hi, shape):
        return jax.random.randint(self._next(), shape, lo, hi, dtype=jnp.int32)

    def uniform(self, shape, lo=0.0, hi=1.0):
        return jax.random.uniform(self._next(), shape, jnp.bfloat16, lo, hi)

    def permutation(self, n):
        return jax.random.permutation(self._next(), n)
kernel_name = 'adaLN_cond__sliding_block_cached__glu_gated_bilinear__decode'

def setup_inputs():
    _rng = _Rng(jax.random.key(int.from_bytes(__import__("os").urandom(4), "little")))
    _w = lambda a: (lambda t: t.astype(jnp.bfloat16) if jnp.issubdtype(t.dtype, jnp.floating) else t)(jnp.asarray(a))

    def _A_setup():
        B, Sq, D = (1, 1, 640)
        Hq, Hkv, Sk, Dh = (32, 32, 32768, 192)
        assert Hq % Hkv == 0, (Hq, Hkv)
        return {'x': _w((lambda *s: _rng.normal(s) * 0.05)(B, Sq, D)), 'k_cache': _w((lambda *s: _rng.normal(s) * 0.05)(B, Hkv, Sk, Dh)), 'v_cache': _w((lambda *s: _rng.normal(s) * 0.05)(B, Hkv, Sk, Dh)), 'wq': _w((lambda *s: _rng.normal(s) * 0.05)(D, Hq * Dh) * D ** (-0.5)), 'wo': _w((lambda *s: _rng.normal(s) * 0.05)(Hq * Dh, D) * (Hq * Dh) ** (-0.5))}
    _A_in = _A_setup()

    def _B_setup():
        B, S, D, F = (1, 1, 640, 1536)
        return {'x': _w((lambda *s: _rng.normal(s) * 0.05)(B, S, D)), 'w_gate': _w((lambda *s: _rng.normal(s) * 0.05)(D, F) * D ** (-0.5)), 'w_up': _w((lambda *s: _rng.normal(s) * 0.05)(D, F) * D ** (-0.5)), 'w_down': _w((lambda *s: _rng.normal(s) * 0.05)(F, D) * F ** (-0.5))}
    _B_in = _B_setup()
    return {'A_x': _A_in['x'], 'A_k_cache': _A_in['k_cache'], 'A_v_cache': _A_in['v_cache'], 'A_wq': _A_in['wq'], 'A_wo': _A_in['wo'], 'B_x': _B_in['x'], 'B_w_gate': _B_in['w_gate'], 'B_w_up': _B_in['w_up'], 'B_w_down': _B_in['w_down'], 'c': _w((lambda *s: _rng.normal(s) * 0.05)(1, 640)), 'w_mod': _w((lambda *s: _rng.normal(s) * 0.05)(640, 6 * 640) * 640 ** (-0.5))}

def reference(A_x, A_k_cache, A_v_cache, A_wq, A_wo, B_x, B_w_gate, B_w_up, B_w_down, c, w_mod):

    def _A_ref(x, k_cache, v_cache, wq, wo):
        B, Sq, D = x.shape
        Hq, Dh = (32, 192)
        Hkv, Sk = (k_cache.shape[1], k_cache.shape[2])
        W = min(4096, max(256, Sk // 4))
        rep = Hq // Hkv
        q = (lambda x, *d: x.transpose(*d))((x @ wq).reshape(B, Sq, Hq, Dh), 0, 2, 1, 3)
        k = jnp.repeat(k_cache[:, :, Sk - W:, :], rep, axis=1)
        v = jnp.repeat(v_cache[:, :, Sk - W:, :], rep, axis=1)
        scores = jnp.einsum('bhqd,bhkd->bhqk', q, k) * Dh ** (-0.5)
        p = _softmax(scores, axis=-1)
        o = jnp.einsum('bhqk,bhkd->bhqd', p, v)
        return (lambda x, *d: x.transpose(*d))(o, 0, 2, 1, 3).reshape(B, Sq, Hq * Dh) @ wo

    def _B_ref(x, w_gate, w_up, w_down):
        g = jnp.einsum('bsd,df->bsf', x, w_gate)
        u = jnp.einsum('bsd,df->bsf', x, w_up)
        h = g * u
        return jnp.einsum('bsf,fd->bsd', h, w_down)
    x = A_x
    mod = (_silu(c) @ w_mod).reshape(c.shape[0], 6, 1, -1)
    sa, ca, ga, sb, cb, gb = (mod[:, 0].copy(), mod[:, 1].copy(), mod[:, 2].copy(), mod[:, 3].copy(), mod[:, 4].copy(), mod[:, 5].copy())
    h = _layernorm(x, axis=-1) * (1 + ca) + sa
    x = x + ga * _A_ref(h, A_k_cache, A_v_cache, A_wq, A_wo)
    h = _layernorm(x, axis=-1) * (1 + cb) + sb
    x = x + gb * _B_ref(h, B_w_gate, B_w_up, B_w_down)
    return x
```

```python
import jax
import jax.numpy as jnp
import jax.experimental.pallas as pl
import jax.experimental.pallas.tpu as pltpu

_BF = jnp.bfloat16
_F32 = jnp.float32


def _layernorm(x, eps=1e-5):
    m = jnp.mean(x, axis=-1, keepdims=True)
    d = x - m
    v = jnp.mean(d * d, axis=-1, keepdims=True)
    return d / jnp.sqrt(v + eps)


def _build(D, H, DH, SK, W, F, *, nslot=2, unroll=8, compute=True):
    G = 2 * DH
    NG = H // 2
    NCB = W // 128
    C0 = SK - W
    FG = 256
    NFG = F // FG
    scale = float(DH) ** -0.5

    def kernel(x_hbm, c_hbm, k_hbm, v_hbm, wq_hbm, wo_hbm, wg_hbm, wu_hbm, wd_hbm, wm_hbm,
               o_ref,
               x_v, c_v, kbuf, vbuf, wqbuf, wobuf, wm_v, wg_v, wu_v, wd_v,
               sem_small, sem_kv, sem_w, sem_m, sem_gu, sem_d):

        def start(src, dst, sem, prio):
            pltpu.make_async_copy(src, dst, sem).start(priority=prio)

        def wait_all(buf, sem):
            pltpu.make_async_copy(buf, buf, sem).wait()

        def issue_group(g, slot):
            r0 = pl.multiple_of(g * G, 128)
            for i in range(D // 128):
                for j in range(G // 128):
                    start(wq_hbm.at[pl.ds(i * 128, 128), pl.ds(r0 + j * 128, 128)],
                          wqbuf.at[slot, pl.ds(i * 128, 128), pl.ds(j * 128, 128)],
                          sem_w.at[slot, 0], 0)
                    start(wo_hbm.at[pl.ds(r0 + j * 128, 128), pl.ds(i * 128, 128)],
                          wobuf.at[slot, pl.ds(j * 128, 128), pl.ds(i * 128, 128)],
                          sem_w.at[slot, 1], 1)
            for hh in range(2):
                def body(cb, carry, hh=hh):
                    cc = pl.multiple_of(cb * 128, 128)
                    start(k_hbm.at[pl.ds(r0 + hh * DH, DH), pl.ds(C0 + cc, 128)],
                          kbuf.at[slot, pl.ds(hh * DH, DH), pl.ds(cc, 128)],
                          sem_kv.at[slot, 0], 0)
                    start(v_hbm.at[pl.ds(r0 + hh * DH, DH), pl.ds(C0 + cc, 128)],
                          vbuf.at[slot, pl.ds(hh * DH, DH), pl.ds(cc, 128)],
                          sem_kv.at[slot, 1], 1)
                    return carry
                jax.lax.fori_loop(0, NCB, body, 0, unroll=unroll)

        def issue_mod(pair):
            for j in range(D // 128):
                for i in range(D // 128):
                    for t in range(2):
                        c0 = (2 * pair + t) * D + j * 128
                        start(wm_hbm.at[pl.ds(i * 128, 128), pl.ds(c0, 128)],
                              wm_v.at[pair, pl.ds(i * 128, 128), pl.ds(t * D + j * 128, 128)],
                              sem_m.at[pair], t)

        def issue_ffn():
            for fg in range(NFG):
                for j in range(FG // 128):
                    for i in range(D // 128):
                        c0 = fg * FG + j * 128
                        start(wg_hbm.at[pl.ds(i * 128, 128), pl.ds(c0, 128)],
                              wg_v.at[fg, pl.ds(i * 128, 128), pl.ds(j * 128, 128)],
                              sem_gu.at[fg, 0], 0)
                        start(wu_hbm.at[pl.ds(i * 128, 128), pl.ds(c0, 128)],
                              wu_v.at[fg, pl.ds(i * 128, 128), pl.ds(j * 128, 128)],
                              sem_gu.at[fg, 1], 1)
            for fg in range(NFG):
                for i in range(D // 128):
                    for j in range(FG // 128):
                        start(wd_hbm.at[pl.ds(fg * FG + j * 128, 128), pl.ds(i * 128, 128)],
                              wd_v.at[fg, pl.ds(j * 128, 128), pl.ds(i * 128, 128)],
                              sem_d.at[fg], j % 2)

        start(c_hbm, c_v, sem_small.at[0], 0)
        start(x_hbm, x_v, sem_small.at[1], 1)
        issue_mod(0)

        def pro(s, carry):
            issue_group(s, s)
            return carry
        jax.lax.fori_loop(0, nslot, pro, 0)
        issue_mod(1)
        issue_mod(2)

        wait_all(c_v, sem_small.at[0])
        wait_all(x_v, sem_small.at[1])
        c = jnp.broadcast_to(c_v[...].astype(_F32), (8, D))
        x = jnp.broadcast_to(x_v[...].astype(_F32), (8, D))
        sc = (c * jax.nn.sigmoid(c)).astype(_BF)
        wait_all(wm_v.at[0], sem_m.at[0])
        mod0 = jnp.dot(sc, wm_v[0], preferred_element_type=_F32)
        h1 = (_layernorm(x) * (1.0 + mod0[:, D:]) + mod0[:, :D]).astype(_BF)

        row = jax.lax.broadcasted_iota(jnp.int32, (8, G), 0)
        lane = jax.lax.broadcasted_iota(jnp.int32, (8, G), 1)
        own = (lane >= row * DH) & (lane < (row + 1) * DH)

        def group_body(g, acc):
            slot = g % nslot
            wait_all(wqbuf.at[slot], sem_w.at[slot, 0])
            wait_all(kbuf.at[slot], sem_kv.at[slot, 0])
            if compute:
                q = jnp.dot(h1, wqbuf[slot], preferred_element_type=_F32)
                qd = jnp.where(own, q, 0.0).astype(_BF)
                s = jnp.dot(qd, kbuf[slot], preferred_element_type=_F32) * scale
                m = jnp.max(s, axis=-1, keepdims=True)
                p = jnp.exp(s - m)
                l = jnp.sum(p, axis=-1, keepdims=True)
            wait_all(vbuf.at[slot], sem_kv.at[slot, 1])
            wait_all(wobuf.at[slot], sem_w.at[slot, 1])
            if compute:
                o = jax.lax.dot_general(p.astype(_BF), vbuf[slot], (((1,), (1,)), ((), ())),
                                        preferred_element_type=_F32)
                od = jnp.where(own, o / l, 0.0).astype(_BF)
                acc = acc + jnp.dot(od, wobuf[slot], preferred_element_type=_F32)

            @pl.when(g + nslot < NG)
            def _():
                issue_group(g + nslot, slot)

            @pl.when(g + nslot == NG - 1)
            def _():
                issue_ffn()
            return acc

        acc = jax.lax.fori_loop(0, NG, group_body, jnp.zeros((8, D), _F32))
        attn = jnp.broadcast_to(jnp.sum(acc, axis=0, keepdims=True), (8, D))

        wait_all(wm_v.at[1], sem_m.at[1])
        wait_all(wm_v.at[2], sem_m.at[2])
        mod1 = jnp.dot(sc, wm_v[1], preferred_element_type=_F32)
        mod2 = jnp.dot(sc, wm_v[2], preferred_element_type=_F32)
        x1 = x + mod1[:, :D] * attn
        h2 = (_layernorm(x1) * (1.0 + mod2[:, :D]) + mod1[:, D:]).astype(_BF)

        hs = []
        for fg in range(NFG):
            wait_all(wg_v.at[fg], sem_gu.at[fg, 0])
            wait_all(wu_v.at[fg], sem_gu.at[fg, 1])
            gt = jnp.dot(h2, wg_v[fg], preferred_element_type=_F32)
            up = jnp.dot(h2, wu_v[fg], preferred_element_type=_F32)
            hs.append((gt * up).astype(_BF))
        y = jnp.zeros((8, D), _F32)
        for fg in range(NFG):
            wait_all(wd_v.at[fg], sem_d.at[fg])
            y = y + jnp.dot(hs[fg], wd_v[fg], preferred_element_type=_F32)
        x2 = x1 + mod2[:, D:] * y
        o_ref[...] = x2[0:1, :].astype(o_ref.dtype)

    scratch = [
        pltpu.VMEM((1, D), _BF), pltpu.VMEM((1, D), _BF),
        pltpu.VMEM((nslot, G, W), _BF), pltpu.VMEM((nslot, G, W), _BF),
        pltpu.VMEM((nslot, D, G), _BF), pltpu.VMEM((nslot, G, D), _BF),
        pltpu.VMEM((3, D, 2 * D), _BF),
        pltpu.VMEM((NFG, D, FG), _BF), pltpu.VMEM((NFG, D, FG), _BF), pltpu.VMEM((NFG, FG, D), _BF),
        pltpu.SemaphoreType.DMA((2,)),
        pltpu.SemaphoreType.DMA((nslot, 2)),
        pltpu.SemaphoreType.DMA((nslot, 2)),
        pltpu.SemaphoreType.DMA((3,)),
        pltpu.SemaphoreType.DMA((NFG, 2)),
        pltpu.SemaphoreType.DMA((NFG,)),
    ]
    return kernel, scratch


def _run(A_x, A_k_cache, A_v_cache, A_wq, A_wo, B_x, B_w_gate, B_w_up, B_w_down, c, w_mod, **kw):
    B, Sq, D = A_x.shape
    _, H, SK, DH = A_k_cache.shape
    F = B_w_gate.shape[1]
    W = min(4096, max(256, SK // 4))
    assert B == 1 and Sq == 1 and A_wq.shape == (D, H * DH)
    kt = jnp.swapaxes(A_k_cache, 2, 3).reshape(H * DH, SK)
    vt = jnp.swapaxes(A_v_cache, 2, 3).reshape(H * DH, SK)
    kernel, scratch = _build(D, H, DH, SK, W, F, **kw)
    out = pl.pallas_call(
        kernel,
        in_specs=[pl.BlockSpec(memory_space=pl.ANY)] * 10,
        out_specs=pl.BlockSpec(memory_space=pltpu.VMEM),
        out_shape=jax.ShapeDtypeStruct((1, D), A_x.dtype),
        scratch_shapes=scratch,
        compiler_params=pltpu.CompilerParams(vmem_limit_bytes=100 * 1024 * 1024),
    )(A_x.reshape(1, D), c, kt, vt, A_wq, A_wo, B_w_gate, B_w_up, B_w_down, w_mod)
    return out.reshape(B, Sq, D)


@jax.jit
def pallas_adaLN_cond__sliding_block_cached__glu_gated_bilinear__decode_kernel(
    A_x: jax.Array,
    A_k_cache: jax.Array,
    A_v_cache: jax.Array,
    A_wq: jax.Array,
    A_wo: jax.Array,
    B_x: jax.Array,
    B_w_gate: jax.Array,
    B_w_up: jax.Array,
    B_w_down: jax.Array,
    c: jax.Array,
    w_mod: jax.Array,
):
    return _run(A_x, A_k_cache, A_v_cache, A_wq, A_wo, B_x, B_w_gate, B_w_up, B_w_down, c, w_mod)
```

```python
import jax
import jax.numpy as jnp
import jax.experimental.pallas as pl
import jax.experimental.pallas.tpu as pltpu

_BF = jnp.bfloat16
_F32 = jnp.float32


def _layernorm(x, eps=1e-5):
    m = jnp.mean(x, axis=-1, keepdims=True)
    d = x - m
    v = jnp.mean(d * d, axis=-1, keepdims=True)
    return d / jnp.sqrt(v + eps)


def _build(D, H, DH, SK, W, F, *, kv_tile=(64, 256), compute=True,
           wm_cfg=(8, 1920, 8), wq_cfg=(8, 2048, 8), wo_cfg=(32, 640, 8), gu_cfg=(16, 1536, 4),
           wd_cfg=(32, 4, 128), trace=False):
    G = 2 * DH
    NG = H // 2
    PW = W // 2
    C0 = SK - W
    scale = float(DH) ** -0.5
    wd_tr, wd_ns, wd_blk = wd_cfg
    wd_len = F // wd_ns
    ND = wd_len // wd_blk

    def kernel(x_hbm, c_hbm, k_hbm, v_hbm, wq_hbm, wo_hbm, wg_hbm, wu_hbm, wd_hbm, wm_hbm,
               o_ref,
               x_v, c_v, kbuf, vbuf, wq_v, wo_v, wm_v, wg_v, wu_v, wd_v, q_s,
               sems):
        S_C, S_X, S_WM, S_WQ, S_WO, S_WG, S_WU, S_KV, S_WD = 0, 1, 2, 3, 4, 5, 6, 7, 11

        def start(src, dst, sem, prio):
            pltpu.make_async_copy(src, dst, sems.at[sem]).start(priority=prio)

        def wait_all(buf, sem, name="w"):
            if trace:
                with jax.named_scope("wait_" + name):
                    pltpu.make_async_copy(buf, buf, sems.at[sem]).wait()
            else:
                pltpu.make_async_copy(buf, buf, sems.at[sem]).wait()

        def stream_steps(pairs, cfg, lo, hi):
            tr, tc, ns = cfg

            def body(i, carry):
                order = list(range(ns))
                if pairs[0][3] is None:
                    order = [s for j in range(ns // 2) for s in (j, ns // 2 + j)]
                for c in range(0, pairs[0][0].shape[1], tc):
                    for s in order:
                        for src, dst, sem, queue in pairs:
                            rows = src.shape[0] // ns
                            r = pl.multiple_of(s * rows + i * tr, 8)
                            start(src.at[pl.ds(r, tr), pl.ds(c, tc)], dst.at[pl.ds(r, tr), pl.ds(c, tc)], sem,
                                  (2 * s) // ns if queue is None else queue)
                return carry
            jax.lax.fori_loop(lo, hi, body, 0)

        def nsteps(ref, cfg):
            return ref.shape[0] // cfg[2] // cfg[0]

        def issue_unit(g, part):
            r0 = g * G if isinstance(g, int) else pl.multiple_of(g * G, 128)
            tr, tc = kv_tile
            for hh in range(2):
                for c in range(0, PW, tc):
                    for r in range(hh * DH, (hh + 1) * DH, tr):
                        for t, (src, dst) in enumerate(((k_hbm, kbuf), (v_hbm, vbuf))):
                            start(src.at[pl.ds(r0 + r, tr), pl.ds(C0 + part * PW + c, tc)],
                                  dst.at[part, pl.ds(r, tr), pl.ds(c, tc)], S_KV + 2 * part + t, t)

        def issue_wd(j):
            for r in range(0, wd_blk, wd_tr):
                for s in [s for i in range(wd_ns // 2) for s in (i, wd_ns // 2 + i)]:
                    start(wd_hbm.at[pl.ds(s * wd_len + j * wd_blk + r, wd_tr), :],
                          wd_v.at[j, pl.ds(s * wd_blk + r, wd_tr), :], S_WD + j, (2 * s) // wd_ns)

        start(c_hbm, c_v, S_C, 0)
        start(x_hbm, x_v, S_X, 1)
        wm_p = [(wm_hbm, wm_v, S_WM, None)]
        wq_p = [(wq_hbm, wq_v, S_WQ, None)]
        wo_p = [(wo_hbm, wo_v, S_WO, None)]
        gu_p = [(wg_hbm, wg_v, S_WG, 0), (wu_hbm, wu_v, S_WU, 1)]
        n_wq, n_wo, n_gu = nsteps(wq_v, wq_cfg), nsteps(wo_v, wo_cfg), nsteps(wg_v, gu_cfg)
        stream_steps(wm_p, wm_cfg, 0, nsteps(wm_v, wm_cfg))
        stream_steps(wq_p, wq_cfg, 0, n_wq // 2)

        wait_all(c_v, S_C, "c")
        wait_all(x_v, S_X, "x")
        c = jnp.broadcast_to(c_v[...].astype(_F32), (8, D))
        x = jnp.broadcast_to(x_v[...].astype(_F32), (8, D))
        sc = (c * jax.nn.sigmoid(c)).astype(_BF)
        wait_all(wm_v, S_WM, "wm")
        mod = jnp.dot(sc, wm_v[...], preferred_element_type=_F32)
        h1 = (_layernorm(x) * (1.0 + mod[:, D:2 * D]) + mod[:, :D]).astype(_BF)

        stream_steps(wq_p, wq_cfg, n_wq // 2, n_wq)
        stream_steps(wo_p, wo_cfg, 0, n_wo // 2)

        row = jax.lax.broadcasted_iota(jnp.int32, (8, G), 0)
        lane = jax.lax.broadcasted_iota(jnp.int32, (8, G), 1)
        own = (lane >= row * DH) & (lane < (row + 1) * DH)

        wait_all(wq_v, S_WQ, "wq")
        for g in range(NG):
            q = jnp.dot(h1, wq_v[:, g * G:(g + 1) * G], preferred_element_type=_F32)
            q_s[g] = jnp.where(own, q, 0.0)

        stream_steps(wo_p, wo_cfg, n_wo // 2, n_wo)
        issue_unit(0, 0)
        issue_unit(0, 1)
        wait_all(wo_v, S_WO, "wo")

        def group(g, acc, last):
            m = l = o = None
            qd = q_s[g].astype(_BF)
            for part in range(2):
                wait_all(kbuf.at[part], S_KV + 2 * part, "k%d" % part)
                if compute:
                    s = jnp.dot(qd, kbuf[part], preferred_element_type=_F32) * scale
                    mp = jnp.max(s, axis=-1, keepdims=True)
                    mn = mp if part == 0 else jnp.maximum(m, mp)
                    p = jnp.exp(s - mn)
                    lp = jnp.sum(p, axis=-1, keepdims=True)
                    pb = p.astype(_BF)
                wait_all(vbuf.at[part], S_KV + 2 * part + 1, "v%d" % part)
                if last and part == 1:
                    stream_steps(gu_p, gu_cfg, n_gu - n_gu // 5, n_gu)
                if compute:
                    op = jax.lax.dot_general(pb, vbuf[part], (((1,), (1,)), ((), ())),
                                             preferred_element_type=_F32)
                    if part == 0:
                        l, o = lp, op
                    else:
                        a = jnp.exp(m - mn)
                        l, o = a * l + lp, a * o + op
                    m = mn
                if not last:
                    issue_unit(g + 1, part)
                elif part == 0:
                    stream_steps(gu_p, gu_cfg, 0, n_gu - n_gu // 5)
            if compute:
                od = jnp.where(own, o / l, 0.0).astype(_BF)
                r0 = g * G if isinstance(g, int) else pl.multiple_of(g * G, 128)
                acc = acc + jnp.dot(od, wo_v[pl.ds(r0, G), :], preferred_element_type=_F32)
            return acc

        acc = jax.lax.fori_loop(0, NG - 1, lambda g, a: group(g, a, False), jnp.zeros((8, D), _F32))
        acc = group(NG - 1, acc, True)
        attn = jnp.broadcast_to(jnp.sum(acc, axis=0, keepdims=True), (8, D))

        x1 = x + mod[:, 2 * D:3 * D] * attn
        h2 = (_layernorm(x1) * (1.0 + mod[:, 4 * D:5 * D]) + mod[:, 3 * D:4 * D]).astype(_BF)
        for j in range(ND):
            issue_wd(j)

        wait_all(wg_v, S_WG, "g")
        gt = jnp.dot(h2, wg_v[...], preferred_element_type=_F32)
        wait_all(wu_v, S_WU, "u")
        up = jnp.dot(h2, wu_v[...], preferred_element_type=_F32)
        hs = (gt * up).astype(_BF)
        y = jnp.zeros((8, D), _F32)
        for j in range(ND):
            hj = jnp.concatenate(
                [hs[:, s * wd_len + j * wd_blk: s * wd_len + (j + 1) * wd_blk] for s in range(wd_ns)], axis=1)
            wait_all(wd_v.at[j], S_WD + j, "d%d" % j)
            y = y + jnp.dot(hj, wd_v[j], preferred_element_type=_F32)
        x2 = x1 + mod[:, 5 * D:] * y
        o_ref[...] = x2[0:1, :].astype(o_ref.dtype)

    scratch = [
        pltpu.VMEM((1, D), _BF), pltpu.VMEM((1, D), _BF),
        pltpu.VMEM((2, G, PW), _BF), pltpu.VMEM((2, G, PW), _BF),
        pltpu.VMEM((D, H * DH), _BF), pltpu.VMEM((H * DH, D), _BF),
        pltpu.VMEM((D, 6 * D), _BF),
        pltpu.VMEM((D, F), _BF), pltpu.VMEM((D, F), _BF), pltpu.VMEM((ND, wd_ns * wd_blk, D), _BF),
        pltpu.VMEM((NG, 8, G), _F32),
        pltpu.SemaphoreType.DMA((11 + ND,)),
    ]
    return kernel, scratch


def _run(A_x, A_k_cache, A_v_cache, A_wq, A_wo, B_x, B_w_gate, B_w_up, B_w_down, c, w_mod,
         nobc=True, nosc=True, **kw):
    B, Sq, D = A_x.shape
    _, H, SK, DH = A_k_cache.shape
    F = B_w_gate.shape[1]
    W = min(4096, max(256, SK // 4))
    assert B == 1 and Sq == 1 and A_wq.shape == (D, H * DH)
    kt = jnp.swapaxes(A_k_cache, 2, 3).reshape(H * DH, SK)
    vt = jnp.swapaxes(A_v_cache, 2, 3).reshape(H * DH, SK)
    kernel, scratch = _build(D, H, DH, SK, W, F, **kw)
    out = pl.pallas_call(
        kernel,
        in_specs=[pl.BlockSpec(memory_space=pl.ANY)] * 10,
        out_specs=pl.BlockSpec(memory_space=pltpu.VMEM),
        out_shape=jax.ShapeDtypeStruct((1, D), A_x.dtype),
        scratch_shapes=scratch,
        compiler_params=pltpu.CompilerParams(
            vmem_limit_bytes=64 * 1024 * 1024,
            disable_bounds_checks=nobc,
            disable_semaphore_checks=nosc,
        ),
    )(A_x.reshape(1, D), c, kt, vt, A_wq, A_wo, B_w_gate, B_w_up, B_w_down, w_mod)
    return out.reshape(B, Sq, D)


@jax.jit
def pallas_adaLN_cond__sliding_block_cached__glu_gated_bilinear__decode_kernel(
    A_x: jax.Array,
    A_k_cache: jax.Array,
    A_v_cache: jax.Array,
    A_wq: jax.Array,
    A_wo: jax.Array,
    B_x: jax.Array,
    B_w_gate: jax.Array,
    B_w_up: jax.Array,
    B_w_down: jax.Array,
    c: jax.Array,
    w_mod: jax.Array,
):
    return _run(A_x, A_k_cache, A_v_cache, A_wq, A_wo, B_x, B_w_gate, B_w_up, B_w_down, c, w_mod)
```

```python
import jax
import jax.numpy as jnp
import jax.experimental.pallas as pl
import jax.experimental.pallas.tpu as pltpu

_BF = jnp.bfloat16
_F32 = jnp.float32


def _layernorm(x, eps=1e-5):
    m = jnp.mean(x, axis=-1, keepdims=True)
    d = x - m
    v = jnp.mean(d * d, axis=-1, keepdims=True)
    return d / jnp.sqrt(v + eps)


def _build(D, H, DH, SK, W, F, *, kv_tile=(64, 256), compute=True,
           wm_cfg=(8, 1280, 8), wq_cfg=(8, 2048, 8), wo_cfg=(16, 640, 8), gu_cfg=(8, 1536, 4),
           wd_tr=16, vp_rows=128, vp_tr=32, gu_n1=80, gu_n2=16, trace=False):
    C0 = SK - W
    scale = float(DH) ** -0.5
    NB = F // 128
    NV = vp_rows // vp_tr if vp_rows else 0

    q = NB // 4
    wd_q = [[(j, q + j) for j in range(q)], [(2 * q + j, 3 * q + j) for j in range(q)]]

    def kernel(x_hbm, c_hbm, k_hbm, v_hbm, wq_hbm, wo_hbm, wg_hbm, wu_hbm, wd_hbm, wm_hbm,
               o_ref,
               x_v, c_v, kbuf, vbuf, wq_v, wo_v, wm_v, wg_v, wu_v, wd_v, q_s,
               sems):
        S_C, S_X, S_WM, S_WQ, S_WO, S_WG, S_WU, S_KV, S_WD = 0, 1, 2, 3, 4, 5, 6, 7, 11
        S_VP = S_WD + NB

        def start(src, dst, sem, prio):
            pltpu.make_async_copy(src, dst, sems.at[sem]).start(priority=prio)

        def wait_all(buf, sem, name="w"):
            if trace:
                with jax.named_scope("wait_" + name):
                    pltpu.make_async_copy(buf, buf, sems.at[sem]).wait()
            else:
                pltpu.make_async_copy(buf, buf, sems.at[sem]).wait()

        def stream_steps(pairs, cfg, lo, hi):
            tr, tc, ns = cfg
            if lo >= hi:
                return

            def body(i, carry):
                order = list(range(ns))
                if pairs[0][3] is None:
                    order = [s for j in range(ns // 2) for s in (j, ns // 2 + j)]
                for c in range(0, pairs[0][0].shape[1], tc):
                    for s in order:
                        for src, dst, sem, queue in pairs:
                            rows = src.shape[0] // ns
                            r = pl.multiple_of(s * rows + i * tr, 8)
                            start(src.at[pl.ds(r, tr), pl.ds(c, tc)], dst.at[pl.ds(r, tr), pl.ds(c, tc)], sem,
                                  (2 * s) // ns if queue is None else queue)
                return carry
            jax.lax.fori_loop(lo, hi, body, 0)

        def nsteps(ref, cfg):
            return ref.shape[0] // cfg[2] // cfg[0]

        def issue_head(h, slot):
            r0 = h * DH if isinstance(h, int) else pl.multiple_of(h * DH, 64)
            tr, tc = kv_tile
            for c in range(0, W, tc):
                for r in range(0, DH, tr):
                    for t, (src, dst) in enumerate(((k_hbm, kbuf), (v_hbm, vbuf))):
                        start(src.at[pl.ds(r0 + r, tr), pl.ds(C0 + c, tc)],
                              dst.at[slot, pl.ds(r, tr), pl.ds(c, tc)], S_KV + 2 * slot + t, t)

        def issue_wd():
            lists = []
            for t in range(2):
                lst = []
                for blocks in wd_q[t]:
                    main = [b for b in blocks if not (vp_rows and b == NB - 1)]
                    for r in range(0, 128, wd_tr):
                        for b in main:
                            lst.append((b * 128 + r, wd_tr, S_WD + b))
                    if len(main) < len(blocks):
                        for r in range(0, 128 - vp_rows, wd_tr):
                            lst.append(((NB - 1) * 128 + r, wd_tr, S_WD + NB - 1))
                        for i in range(NV):
                            for r in range(0, vp_tr, wd_tr):
                                lst.append((F - vp_rows + i * vp_tr + r, wd_tr, S_VP + i))
                lists.append(lst)
            for i in range(max(len(l) for l in lists)):
                for t in range(2):
                    if i < len(lists[t]):
                        r, n, sem = lists[t][i]
                        start(wd_hbm.at[pl.ds(r, n), :], wd_v.at[pl.ds(r, n), :], sem, t)

        start(c_hbm, c_v, S_C, 0)
        start(x_hbm, x_v, S_X, 1)
        wm_p = [(wm_hbm, wm_v, S_WM, None)]
        wq_p = [(wq_hbm, wq_v, S_WQ, None)]
        wo_p = [(wo_hbm, wo_v, S_WO, None)]
        gu_p = [(wg_hbm, wg_v, S_WG, 0), (wu_hbm, wu_v, S_WU, 1)]
        n_wq, n_wo, n_gu = nsteps(wq_v, wq_cfg), nsteps(wo_v, wo_cfg), nsteps(wg_v, gu_cfg)
        gu_per = 2 * gu_cfg[2] * (F // gu_cfg[1])
        gu_a = min(n_gu, gu_n1 // gu_per)
        gu_b = min(n_gu, (gu_n1 + gu_n2) // gu_per)
        stream_steps(wm_p, wm_cfg, 0, nsteps(wm_v, wm_cfg))
        stream_steps(wq_p, wq_cfg, 0, n_wq // 2)

        wait_all(c_v, S_C, "c")
        wait_all(x_v, S_X, "x")
        c = jnp.broadcast_to(c_v[...].astype(_F32), (8, D))
        x = jnp.broadcast_to(x_v[...].astype(_F32), (8, D))
        sc = (c * jax.nn.sigmoid(c)).astype(_BF)
        wait_all(wm_v, S_WM, "wm")
        mod = jnp.dot(sc, wm_v[...], preferred_element_type=_F32)
        h1 = (_layernorm(x) * (1.0 + mod[:, D:2 * D]) + mod[:, :D]).astype(_BF)

        stream_steps(wq_p, wq_cfg, n_wq // 2, n_wq)
        stream_steps(wo_p, wo_cfg, 0, n_wo)
        issue_head(0, 0)

        wait_all(wq_v, S_WQ, "wq")
        for g in range(H // 2):
            q2 = jnp.dot(h1, wq_v[:, 2 * g * DH:(2 * g + 2) * DH], preferred_element_type=_F32)
            q_s[2 * g] = q2[:, :DH]
            q_s[2 * g + 1] = q2[:, DH:]

        issue_head(1, 1)
        wait_all(wo_v, S_WO, "wo")

        def head(h, slot, acc, tail):
            wait_all(kbuf.at[slot], S_KV + 2 * slot, "k%d" % slot)
            if compute:
                s = jnp.dot(q_s[h].astype(_BF), kbuf[slot], preferred_element_type=_F32) * scale
                p = jnp.exp(s - jnp.max(s, axis=-1, keepdims=True))
                l = jnp.sum(p, axis=-1, keepdims=True)
                pb = p.astype(_BF)
            wait_all(vbuf.at[slot], S_KV + 2 * slot + 1, "v%d" % slot)
            if tail == 2:
                stream_steps(gu_p, gu_cfg, gu_a, gu_b)
            if compute:
                o = jax.lax.dot_general(pb, vbuf[slot], (((1,), (1,)), ((), ())),
                                        preferred_element_type=_F32)
            if tail == 0:
                issue_head(h + 2, slot)
            elif tail == 1:
                stream_steps(gu_p, gu_cfg, 0, gu_a)
            if compute:
                r0 = h * DH if isinstance(h, int) else pl.multiple_of(h * DH, 64)
                acc = acc + jnp.dot((o / l).astype(_BF), wo_v[pl.ds(r0, DH), :],
                                    preferred_element_type=_F32)
            return acc

        def pair(g, acc):
            return head(2 * g + 1, 1, head(2 * g, 0, acc, 0), 0)

        attn = jax.lax.fori_loop(0, H // 2 - 1, pair, jnp.zeros((8, D), _F32))
        attn = head(H - 1, 1, head(H - 2, 0, attn, 1), 2)

        x1 = x + mod[:, 2 * D:3 * D] * attn
        h2 = (_layernorm(x1) * (1.0 + mod[:, 4 * D:5 * D]) + mod[:, 3 * D:4 * D]).astype(_BF)
        stream_steps(gu_p, gu_cfg, gu_b, n_gu)
        issue_wd()

        wait_all(wg_v, S_WG, "g")
        gt = jnp.dot(h2, wg_v[...], preferred_element_type=_F32)
        wait_all(wu_v, S_WU, "u")
        up = jnp.dot(h2, wu_v[...], preferred_element_type=_F32)
        hs = (gt * up).astype(_BF)
        if vp_rows:
            hcol = jnp.broadcast_to(hs[0:1, F - 128:].astype(_F32), (128, 128)).T

        y = jnp.zeros((8, D), _F32)
        for t in range(2):
            for blocks in wd_q[t]:
                for b in blocks:
                    n = 128 - vp_rows if b == NB - 1 else 128
                    if n:
                        wait_all(wd_v.at[pl.ds(b * 128, n), :], S_WD + b, "d%d" % b)
                for b in blocks:
                    n = 128 - vp_rows if b == NB - 1 else 128
                    if n:
                        y = y + jnp.dot(hs[:, b * 128:b * 128 + n], wd_v[pl.ds(b * 128, n), :],
                                        preferred_element_type=_F32)
        gb = mod[:, 5 * D:]
        x2 = x1 + gb * y
        if vp_rows:
            part = jnp.zeros((8, D), _F32)
            for i in range(NV):
                r = F - vp_rows + i * vp_tr
                wait_all(wd_v.at[pl.ds(r, vp_tr), :], S_VP + i, "p%d" % i)
                w = wd_v[pl.ds(r, vp_tr), :].astype(_F32)
                hc = hcol[r - (F - 128): r - (F - 128) + vp_tr, :]
                prod = w * jnp.concatenate([hc] * (D // 128), axis=1)
                for k in range(vp_tr // 8):
                    part = part + prod[8 * k:8 * k + 8, :]
            x2 = x2[0:1, :] + gb[0:1, :] * jnp.sum(part, axis=0, keepdims=True)
        o_ref[...] = x2[0:1, :].astype(o_ref.dtype)

    scratch = [
        pltpu.VMEM((1, D), _BF), pltpu.VMEM((1, D), _BF),
        pltpu.VMEM((2, DH, W), _BF), pltpu.VMEM((2, DH, W), _BF),
        pltpu.VMEM((D, H * DH), _BF), pltpu.VMEM((H * DH, D), _BF),
        pltpu.VMEM((D, 6 * D), _BF),
        pltpu.VMEM((D, F), _BF), pltpu.VMEM((D, F), _BF), pltpu.VMEM((F, D), _BF),
        pltpu.VMEM((H, 8, DH), _F32),
        pltpu.SemaphoreType.DMA((11 + NB + NV,)),
    ]
    return kernel, scratch


def _run(A_x, A_k_cache, A_v_cache, A_wq, A_wo, B_x, B_w_gate, B_w_up, B_w_down, c, w_mod,
         nobc=True, nosc=True, **kw):
    B, Sq, D = A_x.shape
    _, H, SK, DH = A_k_cache.shape
    F = B_w_gate.shape[1]
    W = min(4096, max(256, SK // 4))
    assert B == 1 and Sq == 1 and A_wq.shape == (D, H * DH)
    kt = jnp.swapaxes(A_k_cache, 2, 3).reshape(H * DH, SK)
    vt = jnp.swapaxes(A_v_cache, 2, 3).reshape(H * DH, SK)
    kernel, scratch = _build(D, H, DH, SK, W, F, **kw)
    out = pl.pallas_call(
        kernel,
        in_specs=[pl.BlockSpec(memory_space=pl.ANY)] * 10,
        out_specs=pl.BlockSpec(memory_space=pltpu.VMEM),
        out_shape=jax.ShapeDtypeStruct((1, D), A_x.dtype),
        scratch_shapes=scratch,
        compiler_params=pltpu.CompilerParams(
            vmem_limit_bytes=64 * 1024 * 1024,
            disable_bounds_checks=nobc,
            disable_semaphore_checks=nosc,
        ),
    )(A_x.reshape(1, D), c, kt, vt, A_wq, A_wo, B_w_gate, B_w_up, B_w_down, w_mod)
    return out.reshape(B, Sq, D)


@jax.jit
def pallas_adaLN_cond__sliding_block_cached__glu_gated_bilinear__decode_kernel(
    A_x: jax.Array,
    A_k_cache: jax.Array,
    A_v_cache: jax.Array,
    A_wq: jax.Array,
    A_wo: jax.Array,
    B_x: jax.Array,
    B_w_gate: jax.Array,
    B_w_up: jax.Array,
    B_w_down: jax.Array,
    c: jax.Array,
    w_mod: jax.Array,
):
    return _run(A_x, A_k_cache, A_v_cache, A_wq, A_wo, B_x, B_w_gate, B_w_up, B_w_down, c, w_mod)
```

```python
import jax
import jax.numpy as jnp
import jax.experimental.pallas as pl
import jax.experimental.pallas.tpu as pltpu

_BF = jnp.bfloat16
_F32 = jnp.float32


def _layernorm(x, eps=1e-5):
    m = jnp.mean(x, axis=-1, keepdims=True)
    d = x - m
    v = jnp.mean(d * d, axis=-1, keepdims=True)
    return d / jnp.sqrt(v + eps)


def _build(D, H, DH, SK, W, F, *, kv_tile=(64, 256), compute=True,
           wm_cfg=(8, 1280, 8), wq_cfg=(8, 2048, 8), wo_cfg=(16, 640, 8), gu_cfg=(8, 1536, 4),
           wd_tr=16, mxu_pairs=((0, 0), (0, 1), (1, 0)), vpu_pairs=((0, 2), (1, 1), (1, 2)), vp_tr=(128, 64, 16),
           gu_n1=80, gu_n2=16, trace=False):
    C0 = SK - W
    scale = float(DH) ** -0.5
    NB = F // 128

    q = NB // 4
    wd_q = [[(j, q + j) for j in range(q)], [(2 * q + j, 3 * q + j) for j in range(q)]]
    assert sorted(mxu_pairs + vpu_pairs) == [(t, j) for t in range(2) for j in range(q)]
    wd_sem = {}
    ngrp = 1
    vpu_groups = []
    for t, j in mxu_pairs:
        for r in range(0, 128, wd_tr):
            wd_sem[t, j, r] = 0
    for (t, j), n in zip(vpu_pairs, vp_tr):
        for r0 in range(0, 128, n):
            for r in range(r0, r0 + n, wd_tr):
                wd_sem[t, j, r] = ngrp
            vpu_groups.append((ngrp, [(b, r0, n) for b in wd_q[t][j]]))
            ngrp += 1
    mxu_blocks = sorted(b for t, j in mxu_pairs for b in wd_q[t][j])
    vpu_blocks = [b for t, j in vpu_pairs for b in wd_q[t][j]]

    def kernel(x_hbm, c_hbm, k_hbm, v_hbm, wq_hbm, wo_hbm, wg_hbm, wu_hbm, wd_hbm, wm_hbm,
               o_ref,
               x_v, c_v, kbuf, vbuf, wq_v, wo_v, wm_v, wg_v, wu_v, wd_v, q_s,
               sems):
        S_C, S_X, S_WM, S_WQ, S_WO, S_WG, S_WU, S_KV, S_WD = 0, 1, 2, 3, 4, 5, 6, 7, 11

        def start(src, dst, sem, prio):
            pltpu.make_async_copy(src, dst, sems.at[sem]).start(priority=prio)

        def wait_all(buf, sem, name="w"):
            if trace:
                with jax.named_scope("wait_" + name):
                    pltpu.make_async_copy(buf, buf, sems.at[sem]).wait()
            else:
                pltpu.make_async_copy(buf, buf, sems.at[sem]).wait()

        def stream_steps(pairs, cfg, lo, hi):
            tr, tc, ns = cfg
            if lo >= hi:
                return

            def body(i, carry):
                order = list(range(ns))
                if pairs[0][3] is None:
                    order = [s for j in range(ns // 2) for s in (j, ns // 2 + j)]
                for c in range(0, pairs[0][0].shape[1], tc):
                    for s in order:
                        for src, dst, sem, queue in pairs:
                            rows = src.shape[0] // ns
                            r = pl.multiple_of(s * rows + i * tr, 8)
                            start(src.at[pl.ds(r, tr), pl.ds(c, tc)], dst.at[pl.ds(r, tr), pl.ds(c, tc)], sem,
                                  (2 * s) // ns if queue is None else queue)
                return carry
            jax.lax.fori_loop(lo, hi, body, 0)

        def nsteps(ref, cfg):
            return ref.shape[0] // cfg[2] // cfg[0]

        def issue_head(h, slot):
            r0 = h * DH if isinstance(h, int) else pl.multiple_of(h * DH, 64)
            tr, tc = kv_tile
            for c in range(0, W, tc):
                for r in range(0, DH, tr):
                    for t, (src, dst) in enumerate(((k_hbm, kbuf), (v_hbm, vbuf))):
                        start(src.at[pl.ds(r0 + r, tr), pl.ds(C0 + c, tc)],
                              dst.at[slot, pl.ds(r, tr), pl.ds(c, tc)], S_KV + 2 * slot + t, t)

        def issue_wd():
            for j in range(q):
                for r in range(0, 128, wd_tr):
                    for i in range(2):
                        for t in range(2):
                            row = wd_q[t][j][i] * 128 + r
                            start(wd_hbm.at[pl.ds(row, wd_tr), :], wd_v.at[pl.ds(row, wd_tr), :],
                                  S_WD + wd_sem[t, j, r], t)

        start(c_hbm, c_v, S_C, 0)
        start(x_hbm, x_v, S_X, 1)
        wm_p = [(wm_hbm, wm_v, S_WM, None)]
        wq_p = [(wq_hbm, wq_v, S_WQ, None)]
        wo_p = [(wo_hbm, wo_v, S_WO, None)]
        gu_p = [(wg_hbm, wg_v, S_WG, 0), (wu_hbm, wu_v, S_WU, 1)]
        n_wq, n_wo, n_gu = nsteps(wq_v, wq_cfg), nsteps(wo_v, wo_cfg), nsteps(wg_v, gu_cfg)
        gu_per = 2 * gu_cfg[2] * (F // gu_cfg[1])
        gu_a = min(n_gu, gu_n1 // gu_per)
        gu_b = min(n_gu, (gu_n1 + gu_n2) // gu_per)
        stream_steps(wm_p, wm_cfg, 0, nsteps(wm_v, wm_cfg))
        stream_steps(wq_p, wq_cfg, 0, n_wq // 2)

        wait_all(c_v, S_C, "c")
        wait_all(x_v, S_X, "x")
        c = jnp.broadcast_to(c_v[...].astype(_F32), (8, D))
        x = jnp.broadcast_to(x_v[...].astype(_F32), (8, D))
        sc = (c * jax.nn.sigmoid(c)).astype(_BF)
        wait_all(wm_v, S_WM, "wm")
        mod = jnp.dot(sc, wm_v[...], preferred_element_type=_F32)
        h1 = (_layernorm(x) * (1.0 + mod[:, D:2 * D]) + mod[:, :D]).astype(_BF)

        stream_steps(wq_p, wq_cfg, n_wq // 2, n_wq)
        stream_steps(wo_p, wo_cfg, 0, n_wo)
        issue_head(0, 0)

        wait_all(wq_v, S_WQ, "wq")
        for g in range(H // 2):
            q2 = jnp.dot(h1, wq_v[:, 2 * g * DH:(2 * g + 2) * DH], preferred_element_type=_F32)
            q_s[2 * g] = q2[:, :DH]
            q_s[2 * g + 1] = q2[:, DH:]

        issue_head(1, 1)
        wait_all(wo_v, S_WO, "wo")

        def head(h, slot, acc, tail):
            wait_all(kbuf.at[slot], S_KV + 2 * slot, "k%d" % slot)
            if compute:
                s = jnp.dot(q_s[h].astype(_BF), kbuf[slot], preferred_element_type=_F32) * scale
                p = jnp.exp(s - jnp.max(s, axis=-1, keepdims=True))
                l = jnp.sum(p, axis=-1, keepdims=True)
                pb = p.astype(_BF)
            wait_all(vbuf.at[slot], S_KV + 2 * slot + 1, "v%d" % slot)
            if tail == 2:
                stream_steps(gu_p, gu_cfg, gu_a, gu_b)
            if compute:
                o = jax.lax.dot_general(pb, vbuf[slot], (((1,), (1,)), ((), ())),
                                        preferred_element_type=_F32)
            if tail == 0:
                issue_head(h + 2, slot)
            elif tail == 1:
                stream_steps(gu_p, gu_cfg, 0, gu_a)
            if compute:
                r0 = h * DH if isinstance(h, int) else pl.multiple_of(h * DH, 64)
                acc = acc + jnp.dot((o / l).astype(_BF), wo_v[pl.ds(r0, DH), :],
                                    preferred_element_type=_F32)
            return acc

        def pair(g, acc):
            return head(2 * g + 1, 1, head(2 * g, 0, acc, 0), 0)

        attn = jax.lax.fori_loop(0, H // 2 - 1, pair, jnp.zeros((8, D), _F32))
        attn = head(H - 1, 1, head(H - 2, 0, attn, 1), 2)

        x1 = x + mod[:, 2 * D:3 * D] * attn
        h2 = (_layernorm(x1) * (1.0 + mod[:, 4 * D:5 * D]) + mod[:, 3 * D:4 * D]).astype(_BF)
        stream_steps(gu_p, gu_cfg, gu_b, n_gu)
        issue_wd()

        wait_all(wg_v, S_WG, "g")
        gt = jnp.dot(h2, wg_v[...], preferred_element_type=_F32)
        wait_all(wu_v, S_WU, "u")
        hs, hcol = {}, {}
        for b in vpu_blocks + mxu_blocks:
            up = jnp.dot(h2, wu_v[:, b * 128:(b + 1) * 128], preferred_element_type=_F32)
            hs[b] = (gt[:, b * 128:(b + 1) * 128] * up).astype(_BF)
            if b in vpu_blocks:
                hcol[b] = jnp.broadcast_to(hs[b][0:1, :].astype(_F32), (128, 128)).T

        for b in mxu_blocks:
            wait_all(wd_v.at[pl.ds(b * 128, 128), :], S_WD, "d%d" % b)
        y = jnp.zeros((8, D), _F32)
        for b in mxu_blocks:
            y = y + jnp.dot(hs[b], wd_v[pl.ds(b * 128, 128), :], preferred_element_type=_F32)
        gb = mod[:, 5 * D:]
        x2 = x1 + gb * y
        part = jnp.zeros((8, D), _F32)
        for grp, pieces in vpu_groups:
            for b, r0, n in pieces:
                wait_all(wd_v.at[pl.ds(b * 128 + r0, n), :], S_WD + grp, "p%d" % grp)
            for b, r0, n in pieces:
                w = wd_v[pl.ds(b * 128 + r0, n), :].astype(_F32)
                prod = w * jnp.concatenate([hcol[b][r0:r0 + n, :]] * (D // 128), axis=1)
                for k in range(n // 8):
                    part = part + prod[8 * k:8 * k + 8, :]
        x2 = x2[0:1, :] + gb[0:1, :] * jnp.sum(part, axis=0, keepdims=True)
        o_ref[...] = x2[0:1, :].astype(o_ref.dtype)

    scratch = [
        pltpu.VMEM((1, D), _BF), pltpu.VMEM((1, D), _BF),
        pltpu.VMEM((2, DH, W), _BF), pltpu.VMEM((2, DH, W), _BF),
        pltpu.VMEM((D, H * DH), _BF), pltpu.VMEM((H * DH, D), _BF),
        pltpu.VMEM((D, 6 * D), _BF),
        pltpu.VMEM((D, F), _BF), pltpu.VMEM((D, F), _BF), pltpu.VMEM((F, D), _BF),
        pltpu.VMEM((H, 8, DH), _F32),
        pltpu.SemaphoreType.DMA((11 + ngrp,)),
    ]
    return kernel, scratch


def _run(A_x, A_k_cache, A_v_cache, A_wq, A_wo, B_x, B_w_gate, B_w_up, B_w_down, c, w_mod,
         nobc=True, nosc=True, **kw):
    B, Sq, D = A_x.shape
    _, H, SK, DH = A_k_cache.shape
    F = B_w_gate.shape[1]
    W = min(4096, max(256, SK // 4))
    assert B == 1 and Sq == 1 and A_wq.shape == (D, H * DH)
    kt = jnp.swapaxes(A_k_cache, 2, 3).reshape(H * DH, SK)
    vt = jnp.swapaxes(A_v_cache, 2, 3).reshape(H * DH, SK)
    kernel, scratch = _build(D, H, DH, SK, W, F, **kw)
    out = pl.pallas_call(
        kernel,
        in_specs=[pl.BlockSpec(memory_space=pl.ANY)] * 10,
        out_specs=pl.BlockSpec(memory_space=pltpu.VMEM),
        out_shape=jax.ShapeDtypeStruct((1, D), A_x.dtype),
        scratch_shapes=scratch,
        compiler_params=pltpu.CompilerParams(
            vmem_limit_bytes=64 * 1024 * 1024,
            disable_bounds_checks=nobc,
            disable_semaphore_checks=nosc,
        ),
    )(A_x.reshape(1, D), c, kt, vt, A_wq, A_wo, B_w_gate, B_w_up, B_w_down, w_mod)
    return out.reshape(B, Sq, D)


@jax.jit
def pallas_adaLN_cond__sliding_block_cached__glu_gated_bilinear__decode_kernel(
    A_x: jax.Array,
    A_k_cache: jax.Array,
    A_v_cache: jax.Array,
    A_wq: jax.Array,
    A_wo: jax.Array,
    B_x: jax.Array,
    B_w_gate: jax.Array,
    B_w_up: jax.Array,
    B_w_down: jax.Array,
    c: jax.Array,
    w_mod: jax.Array,
):
    return _run(A_x, A_k_cache, A_v_cache, A_wq, A_wo, B_x, B_w_gate, B_w_up, B_w_down, c, w_mod)
```

```python
import jax
import jax.numpy as jnp
import jax.experimental.pallas as pl
import jax.experimental.pallas.tpu as pltpu

_BF = jnp.bfloat16
_F32 = jnp.float32


def _layernorm(x, eps=1e-5):
    m = jnp.mean(x, axis=-1, keepdims=True)
    d = x - m
    v = jnp.mean(d * d, axis=-1, keepdims=True)
    return d / jnp.sqrt(v + eps)


def _build(D, H, DH, SK, W, F):
    C0 = SK - W
    scale = float(DH) ** -0.5
    KV_TILE = (64, 256)
    WM, WQ, WO, GU = (8, 2 * D, 8), (8, 2048, 8), (16, D, 8), (8, F, 4)
    GU_A, GU_B = 10, 12
    WD_TR = 16

    HF = F // 2
    wd_mxu = [(0, 512), (HF, 256)]
    wd_vpu = ([(512, 128), (HF + 256, 128), (640, 128), (HF + 384, 128), (HF + 512, 64), (HF + 576, 64)]
              + [(HF + 640 + r, 16) for r in range(0, 128, 16)])
    wd_groups = wd_mxu + wd_vpu
    assert sorted(r for r0, n in wd_groups for r in range(r0, r0 + n, 8)) == list(range(0, F, 8))
    vpu_blocks = sorted({r0 // 128 for r0, _ in wd_vpu}, key=[r0 // 128 for r0, _ in wd_vpu].index)

    def kernel(x_hbm, c_hbm, k_hbm, v_hbm, wq_hbm, wo_hbm, wg_hbm, wu_hbm, wd_hbm, wm_hbm,
               o_ref,
               x_v, c_v, kbuf, vbuf, wq_v, wo_v, wm_v, wg_v, wu_v, wd_v, q_s, sems):
        S_C, S_X, S_WM, S_WQ, S_WO, S_WG, S_WU, S_KV, S_WD = 0, 1, 2, 3, 4, 5, 6, 7, 11

        def start(src, dst, sem, queue):
            pltpu.make_async_copy(src, dst, sems.at[sem]).start(priority=queue)

        def wait_all(buf, sem):
            pltpu.make_async_copy(buf, buf, sems.at[sem]).wait()

        def stream(mats, cfg, lo, hi, force=None):
            tr, tc, ns = cfg
            order = list(range(ns))
            if mats[0][3] is None:
                order = [s for j in range(ns // 2) for s in (j, ns // 2 + j)]

            def body(i, carry):
                for c in range(0, mats[0][0].shape[1], tc):
                    for s in order:
                        for src, dst, sem, queue in mats:
                            r = pl.multiple_of(s * (src.shape[0] // ns) + i * tr, 8)
                            qn = (2 * s) // ns if queue is None else queue
                            start(src.at[pl.ds(r, tr), pl.ds(c, tc)], dst.at[pl.ds(r, tr), pl.ds(c, tc)],
                                  sem, qn if force is None else force)
                return carry
            jax.lax.fori_loop(lo, hi, body, 0)

        def nsteps(ref, cfg):
            return ref.shape[0] // cfg[2] // cfg[0]

        def head_row(h):
            return h * DH if isinstance(h, int) else pl.multiple_of(h * DH, 64)

        def issue_head(h, slot):
            r0 = head_row(h)
            tr, tc = KV_TILE
            for c in range(0, W, tc):
                for r in range(0, DH, tr):
                    for t, (src, dst) in enumerate(((k_hbm, kbuf), (v_hbm, vbuf))):
                        start(src.at[pl.ds(r0 + r, tr), pl.ds(C0 + c, tc)],
                              dst.at[slot, pl.ds(r, tr), pl.ds(c, tc)], S_KV + 2 * slot + t, t)

        def issue_wd():
            for r in range(0, HF, WD_TR):
                for t in range(2):
                    row = t * HF + r
                    grp = [g for g, (r0, n) in enumerate(wd_groups) if r0 <= row < r0 + n][0]
                    start(wd_hbm.at[pl.ds(row, WD_TR), :], wd_v.at[pl.ds(row, WD_TR), :], S_WD + grp, t)

        wm_m = [(wm_hbm, wm_v, S_WM, None)]
        wq_m = [(wq_hbm, wq_v, S_WQ, None)]
        wo_m = [(wo_hbm, wo_v, S_WO, None)]
        gu_m = [(wg_hbm, wg_v, S_WG, 0), (wu_hbm, wu_v, S_WU, 1)]
        n_wq = nsteps(wq_v, WQ)

        start(c_hbm, c_v, S_C, 0)
        start(x_hbm, x_v, S_X, 1)
        stream(wm_m, WM, 0, 1, force=1)
        stream(wm_m, WM, 1, nsteps(wm_v, WM))
        stream(wq_m, WQ, 0, n_wq // 2)

        wait_all(c_v, S_C)
        wait_all(x_v, S_X)
        c = jnp.broadcast_to(c_v[...].astype(_F32), (8, D))
        x = jnp.broadcast_to(x_v[...].astype(_F32), (8, D))
        sc = (c * jax.nn.sigmoid(c)).astype(_BF)
        wait_all(wm_v, S_WM)
        mod = jnp.dot(sc, wm_v[...], preferred_element_type=_F32)
        h1 = (_layernorm(x) * (1.0 + mod[:, D:2 * D]) + mod[:, :D]).astype(_BF)

        stream(wq_m, WQ, n_wq // 2, n_wq)
        stream(wo_m, WO, 0, nsteps(wo_v, WO))
        issue_head(0, 0)

        wait_all(wq_v, S_WQ)
        for g in range(H // 2):
            q2 = jnp.dot(h1, wq_v[:, 2 * g * DH:(2 * g + 2) * DH], preferred_element_type=_F32)
            q_s[2 * g] = q2[:, :DH]
            q_s[2 * g + 1] = q2[:, DH:]

        issue_head(1, 1)
        wait_all(wo_v, S_WO)

        def head(h, slot, acc, tail):
            wait_all(kbuf.at[slot], S_KV + 2 * slot)
            s = jnp.dot(q_s[h].astype(_BF), kbuf[slot], preferred_element_type=_F32) * scale
            p = jnp.exp(s - jnp.max(s, axis=-1, keepdims=True))
            l = jnp.sum(p, axis=-1, keepdims=True)
            pb = p.astype(_BF)
            wait_all(vbuf.at[slot], S_KV + 2 * slot + 1)
            if tail == 2:
                stream(gu_m, GU, GU_A, GU_B)
            o = jax.lax.dot_general(pb, vbuf[slot], (((1,), (1,)), ((), ())),
                                    preferred_element_type=_F32)
            if tail == 0:
                issue_head(h + 2, slot)
            elif tail == 1:
                stream(gu_m, GU, 0, GU_A)
            return acc + jnp.dot((o / l).astype(_BF), wo_v[pl.ds(head_row(h), DH), :],
                                 preferred_element_type=_F32)

        def pair(g, acc):
            return head(2 * g + 1, 1, head(2 * g, 0, acc, 0), 0)

        attn = jax.lax.fori_loop(0, H // 2 - 1, pair, jnp.zeros((8, D), _F32))
        attn = head(H - 1, 1, head(H - 2, 0, attn, 1), 2)

        x1 = x + mod[:, 2 * D:3 * D] * attn
        h2 = (_layernorm(x1) * (1.0 + mod[:, 4 * D:5 * D]) + mod[:, 3 * D:4 * D]).astype(_BF)
        stream(gu_m, GU, GU_B, nsteps(wg_v, GU))
        issue_wd()

        wait_all(wg_v, S_WG)
        gate = jnp.dot(h2, wg_v[...], preferred_element_type=_F32)
        wait_all(wu_v, S_WU)

        def hidden(c0, n):
            up = jnp.dot(h2, wu_v[:, c0:c0 + n], preferred_element_type=_F32)
            return (gate[:, c0:c0 + n] * up).astype(_BF)

        hcol = {b: jnp.broadcast_to(hidden(b * 128, 128)[0:1, :].astype(_F32), (128, 128)).T
                for b in vpu_blocks}
        hrow = [hidden(r0, n) for r0, n in wd_mxu]

        for g, (r0, n) in enumerate(wd_mxu):
            wait_all(wd_v.at[pl.ds(r0, n), :], S_WD + g)
        y = jnp.zeros((8, D), _F32)
        for hr, (r0, n) in zip(hrow, wd_mxu):
            y = y + jnp.dot(hr, wd_v[pl.ds(r0, n), :], preferred_element_type=_F32)
        gb = mod[0:1, 5 * D:]
        x2 = x1[0:1, :] + gb * y[0:1, :]

        part = jnp.zeros((8, D), _F32)
        for g, (r0, n) in enumerate(wd_vpu):
            wait_all(wd_v.at[pl.ds(r0, n), :], S_WD + len(wd_mxu) + g)
            hc = hcol[r0 // 128][r0 % 128:r0 % 128 + n, :]
            prod = wd_v[pl.ds(r0, n), :].astype(_F32) * jnp.concatenate([hc] * (D // 128), axis=1)
            for k in range(0, n, 8):
                part = part + prod[k:k + 8, :]
        o_ref[...] = (x2 + gb * jnp.sum(part, axis=0, keepdims=True)).astype(o_ref.dtype)

    scratch = [
        pltpu.VMEM((1, D), _BF), pltpu.VMEM((1, D), _BF),
        pltpu.VMEM((2, DH, W), _BF), pltpu.VMEM((2, DH, W), _BF),
        pltpu.VMEM((D, H * DH), _BF), pltpu.VMEM((H * DH, D), _BF),
        pltpu.VMEM((D, 6 * D), _BF),
        pltpu.VMEM((D, F), _BF), pltpu.VMEM((D, F), _BF), pltpu.VMEM((F, D), _BF),
        pltpu.VMEM((H, 8, DH), _F32),
        pltpu.SemaphoreType.DMA((11 + len(wd_groups),)),
    ]
    return kernel, scratch


def _run(A_x, A_k_cache, A_v_cache, A_wq, A_wo, B_x, B_w_gate, B_w_up, B_w_down, c, w_mod):
    B, Sq, D = A_x.shape
    _, H, SK, DH = A_k_cache.shape
    F = B_w_gate.shape[1]
    W = min(4096, max(256, SK // 4))
    assert (B, Sq, D, H, DH, F) == (1, 1, 640, 32, 192, 1536) and A_wq.shape == (D, H * DH)
    kt = jnp.swapaxes(A_k_cache, 2, 3).reshape(H * DH, SK)
    vt = jnp.swapaxes(A_v_cache, 2, 3).reshape(H * DH, SK)
    kernel, scratch = _build(D, H, DH, SK, W, F)
    out = pl.pallas_call(
        kernel,
        in_specs=[pl.BlockSpec(memory_space=pl.ANY)] * 10,
        out_specs=pl.BlockSpec(memory_space=pltpu.VMEM),
        out_shape=jax.ShapeDtypeStruct((1, D), A_x.dtype),
        scratch_shapes=scratch,
        compiler_params=pltpu.CompilerParams(
            vmem_limit_bytes=64 * 1024 * 1024,
            disable_bounds_checks=True,
            disable_semaphore_checks=True,
        ),
    )(A_x.reshape(1, D), c, kt, vt, A_wq, A_wo, B_w_gate, B_w_up, B_w_down, w_mod)
    return out.reshape(B, Sq, D)


@jax.jit
def pallas_adaLN_cond__sliding_block_cached__glu_gated_bilinear__decode_kernel(
    A_x: jax.Array,
    A_k_cache: jax.Array,
    A_v_cache: jax.Array,
    A_wq: jax.Array,
    A_wo: jax.Array,
    B_x: jax.Array,
    B_w_gate: jax.Array,
    B_w_up: jax.Array,
    B_w_down: jax.Array,
    c: jax.Array,
    w_mod: jax.Array,
):
    return _run(A_x, A_k_cache, A_v_cache, A_wq, A_wo, B_x, B_w_gate, B_w_up, B_w_down, c, w_mod)
```

```python
import jax
import jax.numpy as jnp
import jax.experimental.pallas as pl
import jax.experimental.pallas.tpu as pltpu

_BF = jnp.bfloat16
_F32 = jnp.float32


def _layernorm(x, eps=1e-5):
    m = jnp.mean(x, axis=-1, keepdims=True)
    d = x - m
    v = jnp.mean(d * d, axis=-1, keepdims=True)
    return d / jnp.sqrt(v + eps)


def _pieces(ncols, lo, hi, phase):
    tpr = ncols // 128
    cuts = [lo] + [t for t in range(lo + 1, hi) if (t - phase) % 16 == 0] + [hi]
    out = []
    for a, b in zip(cuts[:-1], cuts[1:]):
        slices = []
        while a < b:
            rg, ct = divmod(a, tpr)
            if ct == 0 and b - a >= tpr:
                n = (b - a) // tpr
                slices.append((rg * 8, n * 8, 0, ncols))
                a += n * tpr
            else:
                n = min(tpr - ct, b - a)
                slices.append((rg * 8, 8, ct * 128, n * 128))
                a += n
        out.append(slices)
    return out


def _walk(shape, phase, span, nstreams):
    total = shape[0] // 8 * (shape[1] // 128)
    bounds = [0] + [s * span * 16 + phase for s in range(1, nstreams)] + [total]
    return [_pieces(shape[1], a, b, phase) for a, b in zip(bounds[:-1], bounds[1:])]


def _build(D, H, DH, SK, W, F, ph_wm=1, ph_wq=14, ph_wo=14, ph_gu=0, gu_span=16, gu_a=40, gu_b=50, wq_frac=0.4):
    C0 = SK - W
    scale = float(DH) ** -0.5
    KV_TILE = (64, 256)
    WD_TR = 16

    HF = F // 2
    wd_mxu = [(0, 512), (HF, 256)]
    wd_vpu = ([(512, 128), (HF + 256, 128), (640, 128), (HF + 384, 128), (HF + 512, 64), (HF + 576, 64)]
              + [(HF + 640 + r, 16) for r in range(0, 128, 16)])
    wd_groups = wd_mxu + wd_vpu
    assert sorted(r for r0, n in wd_groups for r in range(r0, r0 + n, 8)) == list(range(0, F, 8))
    vpu_blocks = sorted({r0 // 128 for r0, _ in wd_vpu}, key=[r0 // 128 for r0, _ in wd_vpu].index)

    def kernel(x_hbm, c_hbm, k_hbm, v_hbm, wq_hbm, wo_hbm, wg_hbm, wu_hbm, wd_hbm, wm_hbm,
               o_ref,
               x_v, c_v, kbuf, vbuf, wq_v, wo_v, wm_v, wg_v, wu_v, wd_v, q_s, sems):
        S_C, S_X, S_WM, S_WQ, S_WO, S_WG, S_WU, S_KV, S_WD = 0, 1, 2, 3, 4, 5, 6, 7, 11

        def start(src, dst, sem, queue):
            pltpu.make_async_copy(src, dst, sems.at[sem]).start(priority=queue)

        def wait_all(buf, sem):
            pltpu.make_async_copy(buf, buf, sems.at[sem]).wait()

        def plan(queues):
            per = []
            for t in range(2):
                n = max(len(st) for _, _, _, st in queues[t])
                per.append([(st[i], src, dst, sem, t) for i in range(n)
                            for src, dst, sem, st in queues[t] if i < len(st)])
            return [per[t][i] for i in range(max(map(len, per))) for t in range(2) if i < len(per[t])]

        def split_plan(src, dst, sem, phase):
            span = -(-(src.shape[0] // 8 * (src.shape[1] // 128)) // (16 * 8))
            st = _walk(src.shape, phase, span, 8)
            return plan([[(src, dst, sem, x) for x in st[:4]], [(src, dst, sem, x) for x in st[4:]]])

        def issue(items, warm=0):
            for k, (piece, src, dst, sem, queue) in enumerate(items):
                for r, nr, c0, nc in piece:
                    start(src.at[pl.ds(r, nr), pl.ds(c0, nc)], dst.at[pl.ds(r, nr), pl.ds(c0, nc)],
                          sem, 1 if k < warm else queue)

        def head_row(h):
            return h * DH if isinstance(h, int) else pl.multiple_of(h * DH, 64)

        def issue_head(h, slot):
            r0 = head_row(h)
            tr, tc = KV_TILE
            for c in range(0, W, tc):
                for r in range(0, DH, tr):
                    for t, (src, dst) in enumerate(((k_hbm, kbuf), (v_hbm, vbuf))):
                        start(src.at[pl.ds(r0 + r, tr), pl.ds(C0 + c, tc)],
                              dst.at[slot, pl.ds(r, tr), pl.ds(c, tc)], S_KV + 2 * slot + t, t)

        def issue_wd():
            for r in range(0, HF, WD_TR):
                for t in range(2):
                    row = t * HF + r
                    grp = [g for g, (r0, n) in enumerate(wd_groups) if r0 <= row < r0 + n][0]
                    start(wd_hbm.at[pl.ds(row, WD_TR), :], wd_v.at[pl.ds(row, WD_TR), :], S_WD + grp, t)

        wm_l = split_plan(wm_hbm, wm_v, S_WM, ph_wm)
        wq_l = split_plan(wq_hbm, wq_v, S_WQ, ph_wq)
        wo_l = split_plan(wo_hbm, wo_v, S_WO, ph_wo)
        gu_st = _walk(wg_hbm.shape, ph_gu, gu_span, 4)
        gu_l = plan([[(wg_hbm, wg_v, S_WG, x) for x in gu_st], [(wu_hbm, wu_v, S_WU, x) for x in gu_st]])
        n_wq = int(len(wq_l) * wq_frac) // 2 * 2

        start(c_hbm, c_v, S_C, 0)
        start(x_hbm, x_v, S_X, 1)
        issue(wm_l, warm=12)
        issue(wq_l[:n_wq])

        wait_all(c_v, S_C)
        wait_all(x_v, S_X)
        c = jnp.broadcast_to(c_v[...].astype(_F32), (8, D))
        x = jnp.broadcast_to(x_v[...].astype(_F32), (8, D))
        sc = (c * jax.nn.sigmoid(c)).astype(_BF)
        wait_all(wm_v, S_WM)
        mod = jnp.dot(sc, wm_v[...], preferred_element_type=_F32)
        h1 = (_layernorm(x) * (1.0 + mod[:, D:2 * D]) + mod[:, :D]).astype(_BF)

        issue(wq_l[n_wq:])
        issue(wo_l)
        issue_head(0, 0)

        wait_all(wq_v, S_WQ)
        for g in range(H // 2):
            q2 = jnp.dot(h1, wq_v[:, 2 * g * DH:(2 * g + 2) * DH], preferred_element_type=_F32)
            q_s[2 * g] = q2[:, :DH]
            q_s[2 * g + 1] = q2[:, DH:]

        issue_head(1, 1)
        wait_all(wo_v, S_WO)

        def head(h, slot, acc, tail):
            wait_all(kbuf.at[slot], S_KV + 2 * slot)
            s = jnp.dot(q_s[h].astype(_BF), kbuf[slot], preferred_element_type=_F32) * scale
            p = jnp.exp(s - jnp.max(s, axis=-1, keepdims=True))
            l = jnp.sum(p, axis=-1, keepdims=True)
            pb = p.astype(_BF)
            wait_all(vbuf.at[slot], S_KV + 2 * slot + 1)
            if tail == 2:
                issue(gu_l[gu_a:gu_b])
            o = jax.lax.dot_general(pb, vbuf[slot], (((1,), (1,)), ((), ())),
                                    preferred_element_type=_F32)
            if tail == 0:
                issue_head(h + 2, slot)
            elif tail == 1:
                issue(gu_l[:gu_a])
            return acc + jnp.dot((o / l).astype(_BF), wo_v[pl.ds(head_row(h), DH), :],
                                 preferred_element_type=_F32)

        def pair(g, acc):
            return head(2 * g + 1, 1, head(2 * g, 0, acc, 0), 0)

        attn = jax.lax.fori_loop(0, H // 2 - 1, pair, jnp.zeros((8, D), _F32))
        attn = head(H - 1, 1, head(H - 2, 0, attn, 1), 2)

        x1 = x + mod[:, 2 * D:3 * D] * attn
        h2 = (_layernorm(x1) * (1.0 + mod[:, 4 * D:5 * D]) + mod[:, 3 * D:4 * D]).astype(_BF)
        issue(gu_l[gu_b:])
        issue_wd()

        wait_all(wg_v, S_WG)
        gate = jnp.dot(h2, wg_v[...], preferred_element_type=_F32)
        wait_all(wu_v, S_WU)

        def hidden(c0, n):
            up = jnp.dot(h2, wu_v[:, c0:c0 + n], preferred_element_type=_F32)
            return (gate[:, c0:c0 + n] * up).astype(_BF)

        hcol = {b: jnp.broadcast_to(hidden(b * 128, 128)[0:1, :].astype(_F32), (128, 128)).T
                for b in vpu_blocks}
        hrow = [hidden(r0, n) for r0, n in wd_mxu]

        for g, (r0, n) in enumerate(wd_mxu):
            wait_all(wd_v.at[pl.ds(r0, n), :], S_WD + g)
        y = jnp.zeros((8, D), _F32)
        for hr, (r0, n) in zip(hrow, wd_mxu):
            y = y + jnp.dot(hr, wd_v[pl.ds(r0, n), :], preferred_element_type=_F32)
        gb = mod[0:1, 5 * D:]
        x2 = x1[0:1, :] + gb * y[0:1, :]

        part = jnp.zeros((8, D), _F32)
        for g, (r0, n) in enumerate(wd_vpu):
            wait_all(wd_v.at[pl.ds(r0, n), :], S_WD + len(wd_mxu) + g)
            hc = hcol[r0 // 128][r0 % 128:r0 % 128 + n, :]
            prod = wd_v[pl.ds(r0, n), :].astype(_F32) * jnp.concatenate([hc] * (D // 128), axis=1)
            for k in range(0, n, 8):
                part = part + prod[k:k + 8, :]
        o_ref[...] = (x2 + gb * jnp.sum(part, axis=0, keepdims=True)).astype(o_ref.dtype)

    scratch = [
        pltpu.VMEM((1, D), _BF), pltpu.VMEM((1, D), _BF),
        pltpu.VMEM((2, DH, W), _BF), pltpu.VMEM((2, DH, W), _BF),
        pltpu.VMEM((D, H * DH), _BF), pltpu.VMEM((H * DH, D), _BF),
        pltpu.VMEM((D, 6 * D), _BF),
        pltpu.VMEM((D, F), _BF), pltpu.VMEM((D, F), _BF), pltpu.VMEM((F, D), _BF),
        pltpu.VMEM((H, 8, DH), _F32),
        pltpu.SemaphoreType.DMA((11 + len(wd_groups),)),
    ]
    return kernel, scratch


def _run(A_x, A_k_cache, A_v_cache, A_wq, A_wo, B_x, B_w_gate, B_w_up, B_w_down, c, w_mod, **kw):
    B, Sq, D = A_x.shape
    _, H, SK, DH = A_k_cache.shape
    F = B_w_gate.shape[1]
    W = min(4096, max(256, SK // 4))
    assert (B, Sq, D, H, DH, F) == (1, 1, 640, 32, 192, 1536) and A_wq.shape == (D, H * DH)
    kt = jnp.swapaxes(A_k_cache, 2, 3).reshape(H * DH, SK)
    vt = jnp.swapaxes(A_v_cache, 2, 3).reshape(H * DH, SK)
    kernel, scratch = _build(D, H, DH, SK, W, F, **kw)
    out = pl.pallas_call(
        kernel,
        in_specs=[pl.BlockSpec(memory_space=pl.ANY)] * 10,
        out_specs=pl.BlockSpec(memory_space=pltpu.VMEM),
        out_shape=jax.ShapeDtypeStruct((1, D), A_x.dtype),
        scratch_shapes=scratch,
        compiler_params=pltpu.CompilerParams(
            vmem_limit_bytes=64 * 1024 * 1024,
            disable_bounds_checks=True,
            disable_semaphore_checks=True,
        ),
    )(A_x.reshape(1, D), c, kt, vt, A_wq, A_wo, B_w_gate, B_w_up, B_w_down, w_mod)
    return out.reshape(B, Sq, D)


@jax.jit
def pallas_adaLN_cond__sliding_block_cached__glu_gated_bilinear__decode_kernel(
    A_x: jax.Array,
    A_k_cache: jax.Array,
    A_v_cache: jax.Array,
    A_wq: jax.Array,
    A_wo: jax.Array,
    B_x: jax.Array,
    B_w_gate: jax.Array,
    B_w_up: jax.Array,
    B_w_down: jax.Array,
    c: jax.Array,
    w_mod: jax.Array,
):
    return _run(A_x, A_k_cache, A_v_cache, A_wq, A_wo, B_x, B_w_gate, B_w_up, B_w_down, c, w_mod)
```

```python
import jax
import jax.numpy as jnp
import jax.experimental.pallas as pl
import jax.experimental.pallas.tpu as pltpu

_BF = jnp.bfloat16
_F32 = jnp.float32


def _layernorm(x, eps=1e-5):
    m = jnp.mean(x, axis=-1, keepdims=True)
    d = x - m
    v = jnp.mean(d * d, axis=-1, keepdims=True)
    return d / jnp.sqrt(v + eps)


def _pieces(ncols, lo, hi, phase):
    tpr = ncols // 128
    cuts = [lo] + [t for t in range(lo + 1, hi) if (t - phase) % 16 == 0] + [hi]
    out = []
    for a, b in zip(cuts[:-1], cuts[1:]):
        slices = []
        while a < b:
            rg, ct = divmod(a, tpr)
            if ct == 0 and b - a >= tpr:
                n = (b - a) // tpr
                slices.append((rg * 8, n * 8, 0, ncols))
                a += n * tpr
            else:
                n = min(tpr - ct, b - a)
                slices.append((rg * 8, 8, ct * 128, n * 128))
                a += n
        out.append(slices)
    return out


def _walk(shape, phase, span, nstreams):
    total = shape[0] // 8 * (shape[1] // 128)
    bounds = [0] + [s * span * 16 + phase for s in range(1, nstreams)] + [total]
    return [_pieces(shape[1], a, b, phase) for a, b in zip(bounds[:-1], bounds[1:])]


def _build(D, H, DH, SK, W, F):
    C0 = SK - W
    scale = float(DH) ** -0.5
    KV_TILE = (64, 256)
    PH_WM, PH_WQ, PH_WO, PH_GU = 1, 14, 14, 0
    GU_A, GU_B = 40, 50
    WD_TR = 16

    HF = F // 2
    wd_mxu = [(0, 512), (HF, 256)]
    wd_vpu = ([(512, 128), (HF + 256, 128), (640, 128), (HF + 384, 128), (HF + 512, 64), (HF + 576, 64)]
              + [(HF + 640 + r, 16) for r in range(0, 128, 16)])
    wd_groups = wd_mxu + wd_vpu
    assert sorted(r for r0, n in wd_groups for r in range(r0, r0 + n, 8)) == list(range(0, F, 8))
    vpu_blocks = sorted({r0 // 128 for r0, _ in wd_vpu}, key=[r0 // 128 for r0, _ in wd_vpu].index)

    def kernel(x_hbm, c_hbm, k_hbm, v_hbm, wq_hbm, wo_hbm, wg_hbm, wu_hbm, wd_hbm, wm_hbm,
               o_ref,
               x_v, c_v, kbuf, vbuf, wq_v, wo_v, wm_v, wg_v, wu_v, wd_v, q_s, sems):
        S_C, S_X, S_WM, S_WQ, S_WO, S_WG, S_WU, S_KV, S_WD = 0, 1, 2, 3, 4, 5, 6, 7, 11

        def start(src, dst, sem, queue):
            pltpu.make_async_copy(src, dst, sems.at[sem]).start(priority=queue)

        def wait_all(buf, sem):
            pltpu.make_async_copy(buf, buf, sems.at[sem]).wait()

        def plan(queues):
            per = []
            for t in range(2):
                n = max(len(st) for _, _, _, st in queues[t])
                per.append([(st[i], src, dst, sem, t) for i in range(n)
                            for src, dst, sem, st in queues[t] if i < len(st)])
            return [per[t][i] for i in range(max(map(len, per))) for t in range(2) if i < len(per[t])]

        def split_plan(src, dst, sem, phase):
            span = -(-(src.shape[0] // 8 * (src.shape[1] // 128)) // (16 * 8))
            st = _walk(src.shape, phase, span, 8)
            return plan([[(src, dst, sem, x) for x in st[:4]], [(src, dst, sem, x) for x in st[4:]]])

        def issue(items, warm=0):
            for k, (piece, src, dst, sem, queue) in enumerate(items):
                for r, nr, c0, nc in piece:
                    start(src.at[pl.ds(r, nr), pl.ds(c0, nc)], dst.at[pl.ds(r, nr), pl.ds(c0, nc)],
                          sem, 1 if k < warm else queue)

        def head_row(h):
            return h * DH if isinstance(h, int) else pl.multiple_of(h * DH, 64)

        def issue_head(h, slot):
            r0 = head_row(h)
            tr, tc = KV_TILE
            for c0 in range(0, W, tc):
                for r in range(0, DH, tr):
                    for t, (src, dst) in enumerate(((k_hbm, kbuf), (v_hbm, vbuf))):
                        start(src.at[pl.ds(r0 + r, tr), pl.ds(C0 + c0, tc)],
                              dst.at[slot, pl.ds(r, tr), pl.ds(c0, tc)], S_KV + 2 * slot + t, t)

        def issue_wd():
            for r in range(0, HF, WD_TR):
                for t in range(2):
                    row = t * HF + r
                    grp = [g for g, (r0, n) in enumerate(wd_groups) if r0 <= row < r0 + n][0]
                    start(wd_hbm.at[pl.ds(row, WD_TR), :], wd_v.at[pl.ds(row, WD_TR), :], S_WD + grp, t)

        wm_l = split_plan(wm_hbm, wm_v, S_WM, PH_WM)
        wq_l = split_plan(wq_hbm, wq_v, S_WQ, PH_WQ)
        wo_l = split_plan(wo_hbm, wo_v, S_WO, PH_WO)
        gu_st = _walk(wg_hbm.shape, PH_GU, 16, 4)
        gu_l = plan([[(wg_hbm, wg_v, S_WG, x) for x in gu_st], [(wu_hbm, wu_v, S_WU, x) for x in gu_st]])
        n_wq = 96

        start(c_hbm, c_v, S_C, 0)
        start(x_hbm, x_v, S_X, 1)
        issue(wm_l, warm=12)
        issue(wq_l[:n_wq])

        wait_all(c_v, S_C)
        wait_all(x_v, S_X)
        c = jnp.broadcast_to(c_v[...].astype(_F32), (8, D))
        x = jnp.broadcast_to(x_v[...].astype(_F32), (8, D))
        sc = (c * jax.nn.sigmoid(c)).astype(_BF)
        wait_all(wm_v, S_WM)
        mod = jnp.dot(sc, wm_v[...], preferred_element_type=_F32)
        h1 = (_layernorm(x) * (1.0 + mod[:, D:2 * D]) + mod[:, :D]).astype(_BF)

        issue(wq_l[n_wq:])
        issue(wo_l)
        issue_head(0, 0)

        wait_all(wq_v, S_WQ)
        for g in range(H // 2):
            q2 = jnp.dot(h1, wq_v[:, 2 * g * DH:(2 * g + 2) * DH], preferred_element_type=_F32)
            q_s[2 * g] = q2[:, :DH]
            q_s[2 * g + 1] = q2[:, DH:]

        issue_head(1, 1)
        wait_all(wo_v, S_WO)

        def head(h, slot, acc, tail):
            wait_all(kbuf.at[slot], S_KV + 2 * slot)
            s = jnp.dot(q_s[h].astype(_BF), kbuf[slot], preferred_element_type=_F32) * scale
            p = jnp.exp(s - jnp.max(s, axis=-1, keepdims=True))
            l = jnp.sum(p, axis=-1, keepdims=True)
            pb = p.astype(_BF)
            wait_all(vbuf.at[slot], S_KV + 2 * slot + 1)
            if tail == 2:
                issue(gu_l[GU_A:GU_B])
            o = jax.lax.dot_general(pb, vbuf[slot], (((1,), (1,)), ((), ())),
                                    preferred_element_type=_F32)
            if tail == 0:
                issue_head(h + 2, slot)
            elif tail == 1:
                issue(gu_l[:GU_A])
            return acc + jnp.dot((o / l).astype(_BF), wo_v[pl.ds(head_row(h), DH), :],
                                 preferred_element_type=_F32)

        def pair(g, acc):
            return head(2 * g + 1, 1, head(2 * g, 0, acc, 0), 0)

        attn = jax.lax.fori_loop(0, H // 2 - 1, pair, jnp.zeros((8, D), _F32))
        attn = head(H - 1, 1, head(H - 2, 0, attn, 1), 2)

        x1 = x + mod[:, 2 * D:3 * D] * attn
        h2 = (_layernorm(x1) * (1.0 + mod[:, 4 * D:5 * D]) + mod[:, 3 * D:4 * D]).astype(_BF)
        issue(gu_l[GU_B:])
        issue_wd()

        wait_all(wg_v, S_WG)
        gate = jnp.dot(h2, wg_v[...], preferred_element_type=_F32)
        wait_all(wu_v, S_WU)

        def hidden(c0, n):
            up = jnp.dot(h2, wu_v[:, c0:c0 + n], preferred_element_type=_F32)
            return (gate[:, c0:c0 + n] * up).astype(_BF)

        hcol = {b: jnp.broadcast_to(hidden(b * 128, 128)[0:1, :].astype(_F32), (128, 128)).T
                for b in vpu_blocks}
        hrow = [hidden(r0, n) for r0, n in wd_mxu]

        for g, (r0, n) in enumerate(wd_mxu):
            wait_all(wd_v.at[pl.ds(r0, n), :], S_WD + g)
        y = jnp.zeros((8, D), _F32)
        for hr, (r0, n) in zip(hrow, wd_mxu):
            y = y + jnp.dot(hr, wd_v[pl.ds(r0, n), :], preferred_element_type=_F32)
        gb = mod[0:1, 5 * D:]
        x2 = x1[0:1, :] + gb * y[0:1, :]

        part = jnp.zeros((8, D), _F32)
        for g, (r0, n) in enumerate(wd_vpu):
            wait_all(wd_v.at[pl.ds(r0, n), :], S_WD + len(wd_mxu) + g)
            hc = hcol[r0 // 128][r0 % 128:r0 % 128 + n, :]
            prod = wd_v[pl.ds(r0, n), :].astype(_F32) * jnp.concatenate([hc] * (D // 128), axis=1)
            for k in range(0, n, 8):
                part = part + prod[k:k + 8, :]
        o_ref[...] = (x2 + gb * jnp.sum(part, axis=0, keepdims=True)).astype(o_ref.dtype)

    scratch = [
        pltpu.VMEM((1, D), _BF), pltpu.VMEM((1, D), _BF),
        pltpu.VMEM((2, DH, W), _BF), pltpu.VMEM((2, DH, W), _BF),
        pltpu.VMEM((D, H * DH), _BF), pltpu.VMEM((H * DH, D), _BF),
        pltpu.VMEM((D, 6 * D), _BF),
        pltpu.VMEM((D, F), _BF), pltpu.VMEM((D, F), _BF), pltpu.VMEM((F, D), _BF),
        pltpu.VMEM((H, 8, DH), _F32),
        pltpu.SemaphoreType.DMA((11 + len(wd_groups),)),
    ]
    return kernel, scratch


def _run(A_x, A_k_cache, A_v_cache, A_wq, A_wo, B_x, B_w_gate, B_w_up, B_w_down, c, w_mod):
    B, Sq, D = A_x.shape
    _, H, SK, DH = A_k_cache.shape
    F = B_w_gate.shape[1]
    W = min(4096, max(256, SK // 4))
    assert (B, Sq, D, H, DH, F) == (1, 1, 640, 32, 192, 1536) and A_wq.shape == (D, H * DH)
    kt = jnp.swapaxes(A_k_cache, 2, 3).reshape(H * DH, SK)
    vt = jnp.swapaxes(A_v_cache, 2, 3).reshape(H * DH, SK)
    kernel, scratch = _build(D, H, DH, SK, W, F)
    out = pl.pallas_call(
        kernel,
        in_specs=[pl.BlockSpec(memory_space=pl.ANY)] * 10,
        out_specs=pl.BlockSpec(memory_space=pltpu.VMEM),
        out_shape=jax.ShapeDtypeStruct((1, D), A_x.dtype),
        scratch_shapes=scratch,
        compiler_params=pltpu.CompilerParams(
            vmem_limit_bytes=64 * 1024 * 1024,
            disable_bounds_checks=True,
            disable_semaphore_checks=True,
        ),
    )(A_x.reshape(1, D), c, kt, vt, A_wq, A_wo, B_w_gate, B_w_up, B_w_down, w_mod)
    return out.reshape(B, Sq, D)


@jax.jit
def pallas_adaLN_cond__sliding_block_cached__glu_gated_bilinear__decode_kernel(
    A_x: jax.Array,
    A_k_cache: jax.Array,
    A_v_cache: jax.Array,
    A_wq: jax.Array,
    A_wo: jax.Array,
    B_x: jax.Array,
    B_w_gate: jax.Array,
    B_w_up: jax.Array,
    B_w_down: jax.Array,
    c: jax.Array,
    w_mod: jax.Array,
):
    return _run(A_x, A_k_cache, A_v_cache, A_wq, A_wo, B_x, B_w_gate, B_w_up, B_w_down, c, w_mod)
```
